```python
import jax
import jax.numpy as jnp

def _softmax(x, axis=-1):
    return jax.nn.softmax(x, axis=axis)
def _gelu(x):
    return jax.nn.gelu(x, approximate=True)
def _silu(x):
    return jax.nn.silu(x)
def _sigmoid(x):
    return jax.nn.sigmoid(x)
def _layernorm(x, axis=-1, eps=1e-5):
    m = jnp.mean(x, axis=axis, keepdims=True)
    v = jnp.var(x, axis=axis, keepdims=True)
    return (x - m) / jnp.sqrt(v + eps)
def _scatter_add(tgt, idx, src, axis=0):
    return tgt.at[idx].add(src)
def _segment_sum(src, seg, n):
    return jax.ops.segment_sum(src, seg, n)
class _Rng:
    def __init__(self, key):
        self._k = key
    def _next(self):
        self._k, sub = jax.random.split(self._k)
        return sub
    def normal(self, shape):
        return jax.random.normal(self._next(), shape, dtype=jnp.bfloat16)
    def randint(self, lo, hi, shape):
        return jax.random.randint(self._next(), shape, lo, hi, dtype=jnp.int32)
    def uniform(self, shape, lo=0.0, hi=1.0):
        return jax.random.uniform(self._next(), shape, jnp.bfloat16, lo, hi)
    def permutation(self, n):
        return jax.random.permutation(self._next(), n)


kernel_name = 'interleave_layers__sliding_block_cached__dense_activation_gelu__decode'

def _fwd_setup_inputs():
    _rng = _Rng(jax.random.key(int.from_bytes(__import__("os").urandom(4), "little")))
    _w = (lambda a: (lambda t: t.astype(jnp.bfloat16) if jnp.issubdtype(t.dtype, jnp.floating) else t)(jnp.asarray(a)))
    def _A_setup():
        B, Sq, D = 2, 1, 512
        Hq, Hkv, Sk, Dh = 32, 8, 32768, 128
        assert Hq % Hkv == 0, (Hq, Hkv)
        return {
            "x": _w((lambda *s: _rng.normal(s) * 0.05)(B, Sq, D)),
            "k_cache": _w((lambda *s: _rng.normal(s) * 0.05)(B, Hkv, Sk, Dh)),
            "v_cache": _w((lambda *s: _rng.normal(s) * 0.05)(B, Hkv, Sk, Dh)),
            "wq": _w((lambda *s: _rng.normal(s) * 0.05)(D, Hq * Dh) * (D ** -0.5)),
            "wo": _w((lambda *s: _rng.normal(s) * 0.05)(Hq * Dh, D) * ((Hq * Dh) ** -0.5)),
        }
    _A_in = _A_setup()

    def _B_setup():
        B, S, D, F = 2, 1, 512, 1792
        return {
            "x": _w((lambda *s: _rng.normal(s) * 0.05)(B, S, D)),
            "w1": _w((lambda *s: _rng.normal(s) * 0.05)(D, F) * (D ** -0.5)),
            "b1": _w((lambda *s: _rng.normal(s) * 0.05)(F) * 0.01),
            "w2": _w((lambda *s: _rng.normal(s) * 0.05)(F, D) * (F ** -0.5)),
            "b2": _w((lambda *s: _rng.normal(s) * 0.05)(D) * 0.01),
        }
    _B_in = _B_setup()

    return {
        "A_x": _A_in["x"],
        "A_k_cache": _A_in["k_cache"],
        "A_v_cache": _A_in["v_cache"],
        "A_wq": _A_in["wq"],
        "A_wo": _A_in["wo"],
        "B_x": _B_in["x"],
        "B_w1": _B_in["w1"],
        "B_b1": _B_in["b1"],
        "B_w2": _B_in["w2"],
        "B_b2": _B_in["b2"],
    }

def _fwd_reference(A_x, A_k_cache, A_v_cache, A_wq, A_wo, B_x, B_w1, B_b1, B_w2, B_b2):
    def _A_ref(x, k_cache, v_cache, wq, wo):
        B, Sq, D = x.shape
        Hq, Dh = 32, 128
        Hkv, Sk = k_cache.shape[1], k_cache.shape[2]
        W = min(4096, max(256, Sk // 4))
        rep = Hq // Hkv
        q = (lambda x, *d: x.transpose(*d))((x @ wq).reshape(B, Sq, Hq, Dh), 0, 2, 1, 3)
        k = jnp.repeat(k_cache[:, :, Sk - W:, :], rep, axis=1)
        v = jnp.repeat(v_cache[:, :, Sk - W:, :], rep, axis=1)
        scores = jnp.einsum("bhqd,bhkd->bhqk", q, k) * (Dh ** -0.5)
        p = _softmax(scores, axis=-1)
        o = jnp.einsum("bhqk,bhkd->bhqd", p, v)
        return (lambda x, *d: x.transpose(*d))(o, 0, 2, 1, 3).reshape(B, Sq, Hq * Dh) @ wo

    def _B_ref(x, w1, b1, w2, b2):
        h = jnp.einsum("bsd,df->bsf", x, w1) + b1
        h = _gelu(h)
        return jnp.einsum("bsf,fd->bsd", h, w2) + b2

    x = A_x
    x = x + _A_ref(_layernorm(x, axis=-1), A_k_cache, A_v_cache, A_wq, A_wo)
    x = x + _B_ref(_layernorm(x, axis=-1), B_w1, B_b1, B_w2, B_b2)
    x = x + _A_ref(_layernorm(x, axis=-1), A_k_cache, A_v_cache, A_wq, A_wo)
    x = x + _B_ref(_layernorm(x, axis=-1), B_w1, B_b1, B_w2, B_b2)
    return x


def setup_inputs():
    _inp = _fwd_setup_inputs()
    _gk = jax.random.fold_in(jax.random.key(int.from_bytes(__import__("os").urandom(4), "little")), 2**31 - 1)
    _shapes = [[2, 1, 512]]
    _dtypes = ['bfloat16']
    _gks = jax.random.split(_gk, len(_shapes))
    _gs = [jax.random.normal(k, s, dtype=jnp.dtype(d)) * 0.05 for k, s, d in zip(_gks, _shapes, _dtypes)]
    _inp["grad_out"] = _gs[0]
    return _inp

def reference(A_x, A_k_cache, A_v_cache, A_wq, A_wo, B_w1, B_b1, B_w2, B_b2, B_x, grad_out):
    _const = dict(B_x=B_x)
    def _f(*_d):
        return _fwd_reference(**{'A_x': _d[0], 'A_k_cache': _d[1], 'A_v_cache': _d[2], 'A_wq': _d[3], 'A_wo': _d[4], 'B_w1': _d[5], 'B_b1': _d[6], 'B_w2': _d[7], 'B_b2': _d[8], **_const})
    _out, _vjp = jax.vjp(_f, A_x, A_k_cache, A_v_cache, A_wq, A_wo, B_w1, B_b1, B_w2, B_b2)
    _grads = _vjp(grad_out)
    _out0 = jnp.asarray(_out)
    return (_out0, *[jnp.asarray(_g) for _g in _grads])
```

```python
import functools
import math

import jax
import jax.numpy as jnp
from jax import lax
import jax.experimental.pallas as pl
import jax.experimental.pallas.tpu as pltpu

F32 = jnp.float32
BF16 = jnp.bfloat16
_NT = (((1,), (1,)), ((), ()))
_NN = (((1,), (0,)), ((), ()))
_EPS = 1e-5
_GC = math.sqrt(2.0 / math.pi)
_GA = 0.044715


def _dot(a, b, dims=_NN):
    return lax.dot_general(a, b, dims, preferred_element_type=F32)


def _ln(x):
    m = jnp.mean(x, axis=-1, keepdims=True)
    xc = x - m
    v = jnp.mean(xc * xc, axis=-1, keepdims=True)
    rs = lax.rsqrt(v + _EPS)
    return xc * rs, rs


def _ln_bwd(dy, y, rs):
    return rs * (dy - jnp.mean(dy, axis=-1, keepdims=True)
                 - y * jnp.mean(dy * y, axis=-1, keepdims=True))


def _gelu_and_grad(h):
    t = jnp.tanh(_GC * (h + _GA * h * h * h))
    g = 0.5 * h * (1.0 + t)
    dg = 0.5 * (1.0 + t) + 0.5 * h * (1.0 - t * t) * _GC * (1.0 + 3.0 * _GA * h * h)
    return g, dg


def _make_kernel(B, HKV, SK, DH, W, D, HQ, F, ZCH):
    REP = HQ // HKV
    NBH = B * HKV
    ZR = SK - W
    NZ = ZR // ZCH
    scale = DH ** -0.5
    R8 = 8
    assert 2 * REP == R8 and NBH * R8 == 128

    def kernel(x_ref, g_ref, b1_ref, b2_ref,
               k_hbm, v_hbm, wq_hbm, wo_hbm, w1_hbm, w2_hbm,
               out_ref, gx_ref, gb1_ref, gb2_ref,
               gk_hbm, gv_hbm, gwq_hbm, gwo_hbm, gw1_hbm, gw2_hbm,
               kbuf, vbuf, wq_v, wo_v, w1_v, w2_v,
               gwq_v, gwo_v, gw1_v, gw2_v, zbuf,
               q_s, do_s, p_s, ds_s, flat_s,
               ksem, vsem, wsem, zsem, osem):
        wq_cp = pltpu.make_async_copy(wq_hbm, wq_v, wsem.at[0])
        wo_cp = pltpu.make_async_copy(wo_hbm, wo_v, wsem.at[1])
        w1_cp = pltpu.make_async_copy(w1_hbm, w1_v, wsem.at[2])
        w2_cp = pltpu.make_async_copy(w2_hbm, w2_v, wsem.at[3])
        wq_cp.start()

        def k_cp(bh):
            return pltpu.make_async_copy(
                k_hbm.at[bh // HKV, bh % HKV, pl.ds(ZR, W), :], kbuf.at[bh], ksem.at[bh])

        def v_cp(bh):
            return pltpu.make_async_copy(
                v_hbm.at[bh // HKV, bh % HKV, pl.ds(ZR, W), :], vbuf.at[bh], vsem.at[bh])

        for bh in range(NBH):
            k_cp(bh).start()
            v_cp(bh).start()
        wo_cp.start()
        w1_cp.start()
        w2_cp.start()

        zbuf[...] = jnp.zeros_like(zbuf)
        q_s[...] = jnp.zeros_like(q_s)
        do_s[...] = jnp.zeros_like(do_s)

        zero_copies = []
        for dst in (gk_hbm, gv_hbm):
            for bh in range(NBH):
                for c in range(NZ):
                    zero_copies.append(pltpu.make_async_copy(
                        zbuf, dst.at[bh // HKV, bh % HKV, pl.ds(c * ZCH, ZCH), :], zsem))

        def scatter_heads(flat, dst, layer):
            for b in range(B):
                for hq in range(HQ):
                    h, r = hq // REP, hq % REP
                    dst[b * HKV + h, pl.ds(layer * REP + r, 1), :] = (
                        flat[b:b + 1, hq * DH:(hq + 1) * DH])

        def attn_fwd(layer, first):
            def body(bh, carry):
                if first:
                    k_cp(bh).wait()
                    v_cp(bh).wait()
                q = q_s[bh].astype(BF16)
                s = _dot(q, kbuf[bh], _NT) * scale
                m = jnp.max(s, axis=-1, keepdims=True)
                e = jnp.exp(s - m)
                l = jnp.sum(e, axis=-1, keepdims=True)
                p = e / l
                if not first:
                    p_s[pl.ds(pl.multiple_of(bh * R8, R8), R8), :] = p
                o = _dot(p.astype(BF16), vbuf[bh])
                flat_s[bh] = o
                return carry
            if first:
                for bh in range(NBH):
                    body(bh, 0)
            else:
                lax.fori_loop(0, NBH, body, 0)
            rows = []
            for b in range(B):
                pieces = []
                for hq in range(HQ):
                    h, r = hq // REP, hq % REP
                    pieces.append(flat_s[b * HKV + h, pl.ds(layer * REP + r, 1), :])
                rows.append(jnp.concatenate(pieces, axis=1))
            return jnp.concatenate(rows, axis=0)

        def attn_bwd(layer, last):
            def body(bh, carry):
                do = do_s[bh].astype(BF16)
                dp = _dot(do, vbuf[bh], _NT)
                p = p_s[pl.ds(pl.multiple_of(bh * R8, R8), R8), :]
                ds = p * (dp - jnp.sum(p * dp, axis=-1, keepdims=True)) * scale
                if last:
                    ds_s[pl.ds(pl.multiple_of(bh * R8, R8), R8), :] = ds
                dq = _dot(ds.astype(BF16), kbuf[bh])
                flat_s[bh] = dq
                return carry
            lax.fori_loop(0, NBH, body, 0)
            rows = []
            for b in range(B):
                pieces = []
                for hq in range(HQ):
                    h, r = hq // REP, hq % REP
                    pieces.append(flat_s[b * HKV + h, pl.ds(layer * REP + r, 1), :])
                rows.append(jnp.concatenate(pieces, axis=1))
            return jnp.concatenate(rows, axis=0)

        b1 = b1_ref[...].astype(F32)
        b2 = b2_ref[...].astype(F32)

        x0 = x_ref[...].astype(F32)
        n1, rs1 = _ln(x0)
        wq_cp.wait()
        q1 = _dot(n1.astype(BF16), wq_v[...])
        scatter_heads(q1, q_s, 0)
        o1 = attn_fwd(0, True)
        wo_cp.wait()
        w1_cp.wait()
        w2_cp.wait()
        for cp in zero_copies:
            cp.start()
        x1 = x0 + _dot(o1.astype(BF16), wo_v[...])
        n2, rs2 = _ln(x1)
        h1 = _dot(n2.astype(BF16), w1_v[...]) + b1
        g1, dg1 = _gelu_and_grad(h1)
        x2 = x1 + _dot(g1.astype(BF16), w2_v[...]) + b2
        n3, rs3 = _ln(x2)
        q2 = _dot(n3.astype(BF16), wq_v[...])
        scatter_heads(q2, q_s, 1)
        o2 = attn_fwd(1, False)
        x3 = x2 + _dot(o2.astype(BF16), wo_v[...])
        n4, rs4 = _ln(x3)
        h2 = _dot(n4.astype(BF16), w1_v[...]) + b1
        g2, dg2 = _gelu_and_grad(h2)
        x4 = x3 + _dot(g2.astype(BF16), w2_v[...]) + b2
        out_ref[...] = x4.astype(out_ref.dtype)

        dx4 = g_ref[...].astype(F32)
        dh2 = _dot(dx4.astype(BF16), w2_v[...], _NT) * dg2
        dn4 = _dot(dh2.astype(BF16), w1_v[...], _NT)
        dx3 = dx4 + _ln_bwd(dn4, n4, rs4)
        do2 = _dot(dx3.astype(BF16), wo_v[...], _NT)
        scatter_heads(do2, do_s, 1)
        dq2 = attn_bwd(1, False)
        dn3 = _dot(dq2.astype(BF16), wq_v[...], _NT)
        dx2 = dx3 + _ln_bwd(dn3, n3, rs3)
        dh1 = _dot(dx2.astype(BF16), w2_v[...], _NT) * dg1
        dn2 = _dot(dh1.astype(BF16), w1_v[...], _NT)
        dx1 = dx2 + _ln_bwd(dn2, n2, rs2)
        do1 = _dot(dx1.astype(BF16), wo_v[...], _NT)
        scatter_heads(do1, do_s, 0)
        dq1 = attn_bwd(0, True)
        dn1 = _dot(dq1.astype(BF16), wq_v[...], _NT)
        dx0 = dx1 + _ln_bwd(dn1, n1, rs1)
        gx_ref[...] = dx0.astype(gx_ref.dtype)

        ds_t = jnp.transpose(ds_s[...]).astype(BF16)
        p_t = jnp.transpose(p_s[...]).astype(BF16)
        q_all = q_s[...].reshape(NBH * R8, DH)
        do_all = do_s[...].reshape(NBH * R8, DH)
        row_bh = lax.broadcasted_iota(jnp.int32, (NBH * R8, DH), 0) // R8
        out_copies = []
        for bh in range(NBH):
            sel = row_bh == bh
            qb = jnp.where(sel, q_all, 0.0).astype(BF16)
            dob = jnp.where(sel, do_all, 0.0).astype(BF16)
            kbuf[bh] = _dot(ds_t, qb).astype(BF16)
            vbuf[bh] = _dot(p_t, dob).astype(BF16)
            ck = pltpu.make_async_copy(
                kbuf.at[bh], gk_hbm.at[bh // HKV, bh % HKV, pl.ds(ZR, W), :], osem)
            cv = pltpu.make_async_copy(
                vbuf.at[bh], gv_hbm.at[bh // HKV, bh % HKV, pl.ds(ZR, W), :], osem)
            ck.start()
            cv.start()
            out_copies += [ck, cv]

        def outer(a, b):
            a8 = jnp.concatenate([a, jnp.zeros_like(a)], axis=0)
            b8 = jnp.concatenate([b, jnp.zeros_like(b)], axis=0)
            return _dot(jnp.transpose(a8).astype(BF16), b8.astype(BF16))

        gwq_v[...] = outer(jnp.concatenate([n1, n3], 0), jnp.concatenate([dq1, dq2], 0)).astype(BF16)
        gwo_v[...] = outer(jnp.concatenate([o1, o2], 0), jnp.concatenate([dx1, dx3], 0)).astype(BF16)
        gw1_v[...] = outer(jnp.concatenate([n2, n4], 0), jnp.concatenate([dh1, dh2], 0)).astype(BF16)
        gw2_v[...] = outer(jnp.concatenate([g1, g2], 0), jnp.concatenate([dx2, dx4], 0)).astype(BF16)
        gb1_ref[...] = jnp.sum(dh1 + dh2, axis=0, keepdims=True).astype(gb1_ref.dtype)
        gb2_ref[...] = jnp.sum(dx2 + dx4, axis=0, keepdims=True).astype(gb2_ref.dtype)
        for src, dst in ((gwq_v, gwq_hbm), (gwo_v, gwo_hbm), (gw1_v, gw1_hbm), (gw2_v, gw2_hbm)):
            cp = pltpu.make_async_copy(src, dst, osem)
            cp.start()
            out_copies.append(cp)

        for cp in zero_copies:
            cp.wait()
        for cp in out_copies:
            cp.wait()

    return kernel


@jax.jit
def pallas_interleave_layers__sliding_block_cached__dense_activation_gelu__decode_kernel(
    A_x: jax.Array,
    A_k_cache: jax.Array,
    A_v_cache: jax.Array,
    A_wq: jax.Array,
    A_wo: jax.Array,
    B_x: jax.Array,
    B_w1: jax.Array,
    B_b1: jax.Array,
    B_w2: jax.Array,
    B_b2: jax.Array,
    grad_out: jax.Array,
):
    B, SQ, D = A_x.shape
    assert SQ == 1
    _, HKV, SK, DH = A_k_cache.shape
    HQ = A_wq.shape[1] // DH
    F = B_w1.shape[1]
    W = min(4096, max(256, SK // 4))
    ZCH = 4096
    NBH = B * HKV

    kernel = _make_kernel(B, HKV, SK, DH, W, D, HQ, F, ZCH)
    vmem = pl.BlockSpec(memory_space=pltpu.VMEM)
    hbm = pl.BlockSpec(memory_space=pl.ANY)
    bf = A_x.dtype
    outs = pl.pallas_call(
        kernel,
        in_specs=[vmem] * 4 + [hbm] * 6,
        out_specs=[vmem] * 4 + [hbm] * 6,
        out_shape=[
            jax.ShapeDtypeStruct((B, D), bf),
            jax.ShapeDtypeStruct((B, D), bf),
            jax.ShapeDtypeStruct((1, F), bf),
            jax.ShapeDtypeStruct((1, D), bf),
            jax.ShapeDtypeStruct(A_k_cache.shape, bf),
            jax.ShapeDtypeStruct(A_v_cache.shape, bf),
            jax.ShapeDtypeStruct(A_wq.shape, bf),
            jax.ShapeDtypeStruct(A_wo.shape, bf),
            jax.ShapeDtypeStruct(B_w1.shape, bf),
            jax.ShapeDtypeStruct(B_w2.shape, bf),
        ],
        scratch_shapes=[
            pltpu.VMEM((NBH, W, DH), bf),
            pltpu.VMEM((NBH, W, DH), bf),
            pltpu.VMEM(A_wq.shape, bf),
            pltpu.VMEM(A_wo.shape, bf),
            pltpu.VMEM(B_w1.shape, bf),
            pltpu.VMEM(B_w2.shape, bf),
            pltpu.VMEM(A_wq.shape, bf),
            pltpu.VMEM(A_wo.shape, bf),
            pltpu.VMEM(B_w1.shape, bf),
            pltpu.VMEM(B_w2.shape, bf),
            pltpu.VMEM((ZCH, DH), bf),
            pltpu.VMEM((NBH, 8, DH), F32),
            pltpu.VMEM((NBH, 8, DH), F32),
            pltpu.VMEM((NBH * 8, W), F32),
            pltpu.VMEM((NBH * 8, W), F32),
            pltpu.VMEM((NBH, 8, DH), F32),
            pltpu.SemaphoreType.DMA((NBH,)),
            pltpu.SemaphoreType.DMA((NBH,)),
            pltpu.SemaphoreType.DMA((4,)),
            pltpu.SemaphoreType.DMA(()),
            pltpu.SemaphoreType.DMA(()),
        ],
        compiler_params=pltpu.CompilerParams(vmem_limit_bytes=110 * 1024 * 1024),
    )(
        A_x.reshape(B, D), grad_out.reshape(B, D),
        B_b1.reshape(1, F), B_b2.reshape(1, D),
        A_k_cache, A_v_cache, A_wq, A_wo, B_w1, B_w2,
    )
    out, gx, gb1, gb2, gk, gv, gwq, gwo, gw1, gw2 = outs
    return (out.reshape(B, SQ, D), gx.reshape(B, SQ, D), gk, gv, gwq, gwo,
            gw1, gb1.reshape(F), gw2, gb2.reshape(D))
```

```python
import math

import jax
import jax.numpy as jnp
from jax import lax
import jax.experimental.pallas as pl
import jax.experimental.pallas.tpu as pltpu

F32 = jnp.float32
BF16 = jnp.bfloat16
_NT = (((1,), (1,)), ((), ()))
_NN = (((1,), (0,)), ((), ()))
_EPS = 1e-5
_GC = math.sqrt(2.0 / math.pi)
_GA = 0.044715


def _dot(a, b, dims=_NN):
    return lax.dot_general(a, b, dims, preferred_element_type=F32)


def _ln(x):
    m = jnp.mean(x, axis=-1, keepdims=True)
    xc = x - m
    v = jnp.mean(xc * xc, axis=-1, keepdims=True)
    rs = lax.rsqrt(v + _EPS)
    return xc * rs, rs


def _ln_bwd(dy, y, rs):
    return rs * (dy - jnp.mean(dy, axis=-1, keepdims=True)
                 - y * jnp.mean(dy * y, axis=-1, keepdims=True))


def _gelu_and_grad(h):
    t = jnp.tanh(_GC * (h + _GA * h * h * h))
    g = 0.5 * h * (1.0 + t)
    dg = 0.5 * (1.0 + t) + 0.5 * h * (1.0 - t * t) * _GC * (1.0 + 3.0 * _GA * h * h)
    return g, dg


def _make_kernel(B, HKV, SK, DH, W, D, HQ, F, ZCH):
    REP = HQ // HKV
    NBH = B * HKV
    ZR = SK - W
    NZ = ZR // ZCH
    scale = DH ** -0.5
    R8 = 8
    assert 2 * REP == R8 and NBH * R8 == 128

    def kernel(x_hbm, g_hbm, b1_hbm, b2_hbm,
               k_hbm, v_hbm, wq_hbm, wo_hbm, w1_hbm, w2_hbm,
               out_hbm, gx_hbm, gb1_hbm, gb2_hbm,
               gk_hbm, gv_hbm, gwq_hbm, gwo_hbm, gw1_hbm, gw2_hbm,
               kbuf, vbuf, wq_v, wo_v, w1_v, w2_v,
               gwq_v, gwo_v, gw1_v, gw2_v, zbuf,
               q_s, do_s, p_s, ds_s, flat_s,
               x_ref, g_ref, b1_ref, b2_ref, out_ref, gx_ref, gb1_ref, gb2_ref,
               ksem, vsem, wsem, zsem, osem, ssem):
        small_in = [pltpu.make_async_copy(src, dst, ssem.at[i]) for i, (src, dst) in enumerate(
            ((x_hbm, x_ref), (g_hbm, g_ref), (b1_hbm, b1_ref), (b2_hbm, b2_ref)))]
        for cp in small_in:
            cp.start()
        wq_cp = pltpu.make_async_copy(wq_hbm, wq_v, wsem.at[0])
        wo_cp = pltpu.make_async_copy(wo_hbm, wo_v, wsem.at[1])
        w1_cp = pltpu.make_async_copy(w1_hbm, w1_v, wsem.at[2])
        w2_cp = pltpu.make_async_copy(w2_hbm, w2_v, wsem.at[3])
        wq_cp.start()

        def k_cp(bh):
            return pltpu.make_async_copy(
                k_hbm.at[bh // HKV, bh % HKV, pl.ds(ZR, W), :], kbuf.at[bh], ksem.at[bh])

        def v_cp(bh):
            return pltpu.make_async_copy(
                v_hbm.at[bh // HKV, bh % HKV, pl.ds(ZR, W), :], vbuf.at[bh], vsem.at[bh])

        for bh in range(NBH):
            k_cp(bh).start()
            v_cp(bh).start()
        wo_cp.start()
        w1_cp.start()
        w2_cp.start()

        zbuf[...] = jnp.zeros_like(zbuf)
        q_s[...] = jnp.zeros_like(q_s)
        do_s[...] = jnp.zeros_like(do_s)

        zero_copies = []
        for dst in (gk_hbm, gv_hbm):
            for bh in range(NBH):
                for c in range(NZ):
                    zero_copies.append(pltpu.make_async_copy(
                        zbuf, dst.at[bh // HKV, bh % HKV, pl.ds(c * ZCH, ZCH), :], zsem))

        def scatter_heads(flat, dst, layer):
            for b in range(B):
                for hq in range(HQ):
                    h, r = hq // REP, hq % REP
                    dst[b * HKV + h, pl.ds(layer * REP + r, 1), :] = (
                        flat[b:b + 1, hq * DH:(hq + 1) * DH])

        def attn_fwd(layer, first):
            def body(bh, carry):
                q = q_s[bh].astype(BF16)
                s = _dot(q, kbuf[bh], _NT) * scale
                m = jnp.max(s, axis=-1, keepdims=True)
                e = jnp.exp(s - m)
                l = jnp.sum(e, axis=-1, keepdims=True)
                p = e / l
                if not first:
                    p_s[pl.ds(pl.multiple_of(bh * R8, R8), R8), :] = p
                o = _dot(p.astype(BF16), vbuf[bh])
                flat_s[bh] = o
                return carry
            lax.fori_loop(0, NBH, body, 0)
            rows = []
            for b in range(B):
                pieces = []
                for hq in range(HQ):
                    h, r = hq // REP, hq % REP
                    pieces.append(flat_s[b * HKV + h, pl.ds(layer * REP + r, 1), :])
                rows.append(jnp.concatenate(pieces, axis=1))
            return jnp.concatenate(rows, axis=0)

        def attn_bwd(layer, last):
            def body(bh, carry):
                do = do_s[bh].astype(BF16)
                dp = _dot(do, vbuf[bh], _NT)
                p = p_s[pl.ds(pl.multiple_of(bh * R8, R8), R8), :]
                ds = p * (dp - jnp.sum(p * dp, axis=-1, keepdims=True)) * scale
                if last:
                    ds_s[pl.ds(pl.multiple_of(bh * R8, R8), R8), :] = ds
                dq = _dot(ds.astype(BF16), kbuf[bh])
                flat_s[bh] = dq
                return carry
            lax.fori_loop(0, NBH, body, 0)
            rows = []
            for b in range(B):
                pieces = []
                for hq in range(HQ):
                    h, r = hq // REP, hq % REP
                    pieces.append(flat_s[b * HKV + h, pl.ds(layer * REP + r, 1), :])
                rows.append(jnp.concatenate(pieces, axis=1))
            return jnp.concatenate(rows, axis=0)

        for cp in small_in:
            cp.wait()
        for bh in range(NBH):
            k_cp(bh).wait()
            v_cp(bh).wait()
        wo_cp.wait()
        w1_cp.wait()
        w2_cp.wait()
        wq_cp.wait()
        for cp in zero_copies:
            cp.start()

        b1 = b1_ref[...].astype(F32).reshape(1, F)
        b2 = b2_ref[...].astype(F32).reshape(1, D)

        x0 = x_ref[...].astype(F32)
        n1, rs1 = _ln(x0)
        q1 = _dot(n1.astype(BF16), wq_v[...])
        scatter_heads(q1, q_s, 0)
        o1 = attn_fwd(0, True)
        x1 = x0 + _dot(o1.astype(BF16), wo_v[...])
        n2, rs2 = _ln(x1)
        h1 = _dot(n2.astype(BF16), w1_v[...]) + b1
        g1, dg1 = _gelu_and_grad(h1)
        x2 = x1 + _dot(g1.astype(BF16), w2_v[...]) + b2
        n3, rs3 = _ln(x2)
        q2 = _dot(n3.astype(BF16), wq_v[...])
        scatter_heads(q2, q_s, 1)
        o2 = attn_fwd(1, False)
        x3 = x2 + _dot(o2.astype(BF16), wo_v[...])
        n4, rs4 = _ln(x3)
        h2 = _dot(n4.astype(BF16), w1_v[...]) + b1
        g2, dg2 = _gelu_and_grad(h2)
        x4 = x3 + _dot(g2.astype(BF16), w2_v[...]) + b2
        out_ref[...] = x4.astype(out_ref.dtype)
        small_out = [pltpu.make_async_copy(out_ref, out_hbm, ssem.at[4])]
        small_out[0].start()

        dx4 = g_ref[...].astype(F32)
        dh2 = _dot(dx4.astype(BF16), w2_v[...], _NT) * dg2
        dn4 = _dot(dh2.astype(BF16), w1_v[...], _NT)
        dx3 = dx4 + _ln_bwd(dn4, n4, rs4)
        do2 = _dot(dx3.astype(BF16), wo_v[...], _NT)
        scatter_heads(do2, do_s, 1)
        dq2 = attn_bwd(1, False)
        dn3 = _dot(dq2.astype(BF16), wq_v[...], _NT)
        dx2 = dx3 + _ln_bwd(dn3, n3, rs3)
        dh1 = _dot(dx2.astype(BF16), w2_v[...], _NT) * dg1
        dn2 = _dot(dh1.astype(BF16), w1_v[...], _NT)
        dx1 = dx2 + _ln_bwd(dn2, n2, rs2)
        do1 = _dot(dx1.astype(BF16), wo_v[...], _NT)
        scatter_heads(do1, do_s, 0)
        dq1 = attn_bwd(0, True)
        dn1 = _dot(dq1.astype(BF16), wq_v[...], _NT)
        dx0 = dx1 + _ln_bwd(dn1, n1, rs1)
        gx_ref[...] = dx0.astype(gx_ref.dtype)
        gb1_ref[...] = jnp.sum(dh1 + dh2, axis=0).astype(gb1_ref.dtype)
        gb2_ref[...] = jnp.sum(dx2 + dx4, axis=0).astype(gb2_ref.dtype)
        for i, (src, dst) in enumerate(((gx_ref, gx_hbm), (gb1_ref, gb1_hbm), (gb2_ref, gb2_hbm))):
            cp = pltpu.make_async_copy(src, dst, ssem.at[5 + i])
            cp.start()
            small_out.append(cp)

        ds_t = jnp.transpose(ds_s[...]).astype(BF16)
        p_t = jnp.transpose(p_s[...]).astype(BF16)
        q_all = q_s[...].reshape(NBH * R8, DH)
        do_all = do_s[...].reshape(NBH * R8, DH)
        row_bh = lax.broadcasted_iota(jnp.int32, (NBH * R8, DH), 0) // R8
        out_copies = []
        for bh in range(NBH):
            sel = row_bh == bh
            qb = jnp.where(sel, q_all, 0.0).astype(BF16)
            dob = jnp.where(sel, do_all, 0.0).astype(BF16)
            kbuf[bh] = _dot(ds_t, qb).astype(BF16)
            vbuf[bh] = _dot(p_t, dob).astype(BF16)
            ck = pltpu.make_async_copy(
                kbuf.at[bh], gk_hbm.at[bh // HKV, bh % HKV, pl.ds(ZR, W), :], osem)
            cv = pltpu.make_async_copy(
                vbuf.at[bh], gv_hbm.at[bh // HKV, bh % HKV, pl.ds(ZR, W), :], osem)
            ck.start()
            cv.start()
            out_copies += [ck, cv]

        def outer(a, b):
            a8 = jnp.concatenate([a, jnp.zeros_like(a)], axis=0)
            b8 = jnp.concatenate([b, jnp.zeros_like(b)], axis=0)
            return _dot(jnp.transpose(a8).astype(BF16), b8.astype(BF16))

        gwq_v[...] = outer(jnp.concatenate([n1, n3], 0), jnp.concatenate([dq1, dq2], 0)).astype(BF16)
        gwo_v[...] = outer(jnp.concatenate([o1, o2], 0), jnp.concatenate([dx1, dx3], 0)).astype(BF16)
        gw1_v[...] = outer(jnp.concatenate([n2, n4], 0), jnp.concatenate([dh1, dh2], 0)).astype(BF16)
        gw2_v[...] = outer(jnp.concatenate([g1, g2], 0), jnp.concatenate([dx2, dx4], 0)).astype(BF16)
        for src, dst in ((gwq_v, gwq_hbm), (gwo_v, gwo_hbm), (gw1_v, gw1_hbm), (gw2_v, gw2_hbm)):
            cp = pltpu.make_async_copy(src, dst, osem)
            cp.start()
            out_copies.append(cp)

        for cp in zero_copies:
            cp.wait()
        for cp in out_copies:
            cp.wait()
        for cp in small_out:
            cp.wait()

    return kernel


@jax.jit
def pallas_interleave_layers__sliding_block_cached__dense_activation_gelu__decode_kernel(
    A_x: jax.Array,
    A_k_cache: jax.Array,
    A_v_cache: jax.Array,
    A_wq: jax.Array,
    A_wo: jax.Array,
    B_x: jax.Array,
    B_w1: jax.Array,
    B_b1: jax.Array,
    B_w2: jax.Array,
    B_b2: jax.Array,
    grad_out: jax.Array,
):
    B, SQ, D = A_x.shape
    assert SQ == 1
    _, HKV, SK, DH = A_k_cache.shape
    HQ = A_wq.shape[1] // DH
    F = B_w1.shape[1]
    W = min(4096, max(256, SK // 4))
    ZCH = 4096
    NBH = B * HKV

    kernel = _make_kernel(B, HKV, SK, DH, W, D, HQ, F, ZCH)
    hbm = pl.BlockSpec(memory_space=pl.ANY)
    bf = A_x.dtype
    outs = pl.pallas_call(
        kernel,
        in_specs=[hbm] * 10,
        out_specs=[hbm] * 10,
        out_shape=[
            jax.ShapeDtypeStruct((B, D), bf),
            jax.ShapeDtypeStruct((B, D), bf),
            jax.ShapeDtypeStruct(B_b1.shape, bf),
            jax.ShapeDtypeStruct(B_b2.shape, bf),
            jax.ShapeDtypeStruct(A_k_cache.shape, bf),
            jax.ShapeDtypeStruct(A_v_cache.shape, bf),
            jax.ShapeDtypeStruct(A_wq.shape, bf),
            jax.ShapeDtypeStruct(A_wo.shape, bf),
            jax.ShapeDtypeStruct(B_w1.shape, bf),
            jax.ShapeDtypeStruct(B_w2.shape, bf),
        ],
        scratch_shapes=[
            pltpu.VMEM((NBH, W, DH), bf),
            pltpu.VMEM((NBH, W, DH), bf),
            pltpu.VMEM(A_wq.shape, bf),
            pltpu.VMEM(A_wo.shape, bf),
            pltpu.VMEM(B_w1.shape, bf),
            pltpu.VMEM(B_w2.shape, bf),
            pltpu.VMEM(A_wq.shape, bf),
            pltpu.VMEM(A_wo.shape, bf),
            pltpu.VMEM(B_w1.shape, bf),
            pltpu.VMEM(B_w2.shape, bf),
            pltpu.VMEM((ZCH, DH), bf),
            pltpu.VMEM((NBH, 8, DH), F32),
            pltpu.VMEM((NBH, 8, DH), F32),
            pltpu.VMEM((NBH * 8, W), F32),
            pltpu.VMEM((NBH * 8, W), F32),
            pltpu.VMEM((NBH, 8, DH), F32),
            pltpu.VMEM((B, D), bf),
            pltpu.VMEM((B, D), bf),
            pltpu.VMEM(B_b1.shape, bf),
            pltpu.VMEM(B_b2.shape, bf),
            pltpu.VMEM((B, D), bf),
            pltpu.VMEM((B, D), bf),
            pltpu.VMEM(B_b1.shape, bf),
            pltpu.VMEM(B_b2.shape, bf),
            pltpu.SemaphoreType.DMA((NBH,)),
            pltpu.SemaphoreType.DMA((NBH,)),
            pltpu.SemaphoreType.DMA((4,)),
            pltpu.SemaphoreType.DMA(()),
            pltpu.SemaphoreType.DMA(()),
            pltpu.SemaphoreType.DMA((8,)),
        ],
        compiler_params=pltpu.CompilerParams(vmem_limit_bytes=110 * 1024 * 1024),
    )(
        A_x.reshape(B, D), grad_out.reshape(B, D), B_b1, B_b2,
        A_k_cache, A_v_cache, A_wq, A_wo, B_w1, B_w2,
    )
    out, gx, gb1, gb2, gk, gv, gwq, gwo, gw1, gw2 = outs
    return (out.reshape(B, SQ, D), gx.reshape(B, SQ, D), gk, gv, gwq, gwo,
            gw1, gb1, gw2, gb2)
```
